```python
import jax
import jax.numpy as jnp

def _softmax(x, axis=-1):
    return jax.nn.softmax(x, axis=axis)
def _gelu(x):
    return jax.nn.gelu(x, approximate=True)
def _silu(x):
    return jax.nn.silu(x)
def _sigmoid(x):
    return jax.nn.sigmoid(x)
def _layernorm(x, axis=-1, eps=1e-5):
    m = jnp.mean(x, axis=axis, keepdims=True)
    v = jnp.var(x, axis=axis, keepdims=True)
    return (x - m) / jnp.sqrt(v + eps)
def _scatter_add(tgt, idx, src, axis=0):
    return tgt.at[idx].add(src)
def _segment_sum(src, seg, n):
    return jax.ops.segment_sum(src, seg, n)
class _Rng:
    def __init__(self, key):
        self._k = key
    def _next(self):
        self._k, sub = jax.random.split(self._k)
        return sub
    def normal(self, shape):
        return jax.random.normal(self._next(), shape, dtype=jnp.bfloat16)
    def randint(self, lo, hi, shape):
        return jax.random.randint(self._next(), shape, lo, hi, dtype=jnp.int32)
    def uniform(self, shape, lo=0.0, hi=1.0):
        return jax.random.uniform(self._next(), shape, jnp.bfloat16, lo, hi)
    def permutation(self, n):
        return jax.random.permutation(self._next(), n)


kernel_name = 'recurrent_scan__sliding_block_cached__mixer_s_mlp__decode'

def _fwd_setup_inputs():
    _rng = _Rng(jax.random.key(int.from_bytes(__import__("os").urandom(4), "little")))
    _w = (lambda a: (lambda t: t.astype(jnp.bfloat16) if jnp.issubdtype(t.dtype, jnp.floating) else t)(jnp.asarray(a)))
    def _A_setup():
        B, Sq, D = 4, 1, 512
        Hq, Hkv, Sk, Dh = 32, 8, 8192, 128
        assert Hq % Hkv == 0, (Hq, Hkv)
        return {
            "x": _w((lambda *s: _rng.normal(s) * 0.05)(B, Sq, D)),
            "k_cache": _w((lambda *s: _rng.normal(s) * 0.05)(B, Hkv, Sk, Dh)),
            "v_cache": _w((lambda *s: _rng.normal(s) * 0.05)(B, Hkv, Sk, Dh)),
            "wq": _w((lambda *s: _rng.normal(s) * 0.05)(D, Hq * Dh) * (D ** -0.5)),
            "wo": _w((lambda *s: _rng.normal(s) * 0.05)(Hq * Dh, D) * ((Hq * Dh) ** -0.5)),
        }
    _A_in = _A_setup()

    def _B_setup():
        B, S, D, F = 4, 1, 512, 1792
        return {
            "x":  _w((lambda *s: _rng.normal(s) * 0.05)(B, S, D)),
            "w1": _w((lambda *s: _rng.normal(s) * 0.05)(D, D) * (D ** -0.5)),
            "w2": _w((lambda *s: _rng.normal(s) * 0.05)(D, D) * (D ** -0.5)),
            "w3": _w((lambda *s: _rng.normal(s) * 0.05)(D, F) * (D ** -0.5)),
            "w4": _w((lambda *s: _rng.normal(s) * 0.05)(F, D) * (F ** -0.5)),
        }
    _B_in = _B_setup()

    return {
        "A_x": _A_in["x"],
        "A_k_cache": _A_in["k_cache"],
        "A_v_cache": _A_in["v_cache"],
        "A_wq": _A_in["wq"],
        "A_wo": _A_in["wo"],
        "B_x": _B_in["x"],
        "B_w1": _B_in["w1"],
        "B_w2": _B_in["w2"],
        "B_w3": _B_in["w3"],
        "B_w4": _B_in["w4"],
    }

def _fwd_reference(A_x, A_k_cache, A_v_cache, A_wq, A_wo, B_x, B_w1, B_w2, B_w3, B_w4):
    def _A_ref(x, k_cache, v_cache, wq, wo):
        B, Sq, D = x.shape
        Hq, Dh = 32, 128
        Hkv, Sk = k_cache.shape[1], k_cache.shape[2]
        W = min(4096, max(256, Sk // 4))
        rep = Hq // Hkv
        q = (lambda x, *d: x.transpose(*d))((x @ wq).reshape(B, Sq, Hq, Dh), 0, 2, 1, 3)
        k = jnp.repeat(k_cache[:, :, Sk - W:, :], rep, axis=1)
        v = jnp.repeat(v_cache[:, :, Sk - W:, :], rep, axis=1)
        scores = jnp.einsum("bhqd,bhkd->bhqk", q, k) * (Dh ** -0.5)
        p = _softmax(scores, axis=-1)
        o = jnp.einsum("bhqk,bhkd->bhqd", p, v)
        return (lambda x, *d: x.transpose(*d))(o, 0, 2, 1, 3).reshape(B, Sq, Hq * Dh) @ wo

    def _B_ref(x, w1, w2, w3, w4):
        B, S, D = x.shape
        h = _gelu(_layernorm(x, axis=-1) @ w1)
        c = D // 4
        g0 = jnp.pad(h[:, :, 0*c:1*c], ((0, 0), (1, 0), (0, 0)))[:, :S, :]
        g1 = jnp.pad(h[:, :, 1*c:2*c], ((0, 0), (0, 1), (0, 0)))[:, 1:, :]
        g2 = jnp.pad(h[:, :, 2*c:3*c], ((0, 0), (2, 0), (0, 0)))[:, :S, :]
        g3 = jnp.pad(h[:, :, 3*c:   ], ((0, 0), (0, 2), (0, 0)))[:, 2:, :]
        hs = jnp.concatenate([g0, g1, g2, g3], axis=-1) @ w2
        x1 = x + hs
        h2 = _gelu(_layernorm(x1, axis=-1) @ w3) @ w4
        return x1 + h2

    x = A_x
    xn = _layernorm(x, axis=-1)
    s = _A_ref(xn, A_k_cache, A_v_cache, A_wq, A_wo)
    g = _silu(_B_ref(xn, B_w1, B_w2, B_w3, B_w4))
    return x + s * g


def setup_inputs():
    _inp = _fwd_setup_inputs()
    _gk = jax.random.fold_in(jax.random.key(int.from_bytes(__import__("os").urandom(4), "little")), 2**31 - 1)
    _shapes = [[4, 1, 512]]
    _dtypes = ['bfloat16']
    _gks = jax.random.split(_gk, len(_shapes))
    _gs = [jax.random.normal(k, s, dtype=jnp.dtype(d)) * 0.05 for k, s, d in zip(_gks, _shapes, _dtypes)]
    _inp["grad_out"] = _gs[0]
    return _inp

def reference(A_x, A_k_cache, A_v_cache, A_wq, A_wo, B_w3, B_w4, B_x, B_w1, B_w2, grad_out):
    _const = dict(B_x=B_x, B_w1=B_w1, B_w2=B_w2)
    def _f(*_d):
        return _fwd_reference(**{'A_x': _d[0], 'A_k_cache': _d[1], 'A_v_cache': _d[2], 'A_wq': _d[3], 'A_wo': _d[4], 'B_w3': _d[5], 'B_w4': _d[6], **_const})
    _out, _vjp = jax.vjp(_f, A_x, A_k_cache, A_v_cache, A_wq, A_wo, B_w3, B_w4)
    _grads = _vjp(grad_out)
    _out0 = jnp.asarray(_out)
    return (_out0, *[jnp.asarray(_g) for _g in _grads])
```

```python
import functools
import math

import jax
import jax.numpy as jnp
from jax import lax
from jax.experimental import pallas as pl
from jax.experimental.pallas import tpu as pltpu

F32 = jnp.float32
BF16 = jnp.bfloat16

NB, D = 4, 512
HQ, HKV, DH = 32, 8, 128
REP = HQ // HKV
SK = 8192
W = min(4096, max(256, SK // 4))
Z = SK - W
FF = 1792
FB = 256
GW = REP * DH
EPS = 1e-5
SCALE = DH ** -0.5
GELU_C = math.sqrt(2.0 / math.pi)

NT = (((1,), (1,)), ((), ()))
TN = (((0,), (0,)), ((), ()))


def _ln(x):
    m = jnp.mean(x, axis=-1, keepdims=True)
    c = x - m
    rstd = lax.rsqrt(jnp.mean(c * c, axis=-1, keepdims=True) + EPS)
    return c * rstd, rstd


def _ln_bwd(dy, y, rstd):
    return rstd * (dy - jnp.mean(dy, axis=-1, keepdims=True)
                   - y * jnp.mean(dy * y, axis=-1, keepdims=True))


def _mm(a, b, dims=(((1,), (0,)), ((), ()))):
    return lax.dot_general(a, b, dims, preferred_element_type=F32)


def make(zr=64, wr=64, rprio=(0, 1), lead_rows=2048, dw_mode="each"):
    def kernel(x_hbm, k_hbm, v_hbm, wq_hbm, wo_hbm, w3_hbm, w4_hbm, go_hbm,
               out_hbm, dx_hbm, dk_hbm, dv_hbm, dwq_hbm, dwo_hbm, dw3_hbm, dw4_hbm,
               x_v, go_v, k_v, v_v, wq_v, wo_v, w3_v, w4_v,
               out_v, dx_v, dk_v, dv_v, dwq_v, dwo_v, dw3_v, dw4_v,
               z_v, u_s, q_s, do_s, o_s, dq_s, sems):
        rsem, lsem, wsem = sems.at[0], sems.at[1], sems.at[2]

        reads = [pltpu.make_async_copy(s, d, rsem) for s, d in (
            (x_hbm, x_v), (go_hbm, go_v), (w3_hbm, w3_v), (w4_hbm, w4_v),
            (wq_hbm, wq_v), (wo_hbm, wo_v))]
        for b in range(NB):
            reads.append(pltpu.make_async_copy(k_hbm.at[b, :, pl.ds(Z, W)], k_v.at[b], rsem))
            if b < NB - 1:
                reads.append(pltpu.make_async_copy(v_hbm.at[b, :, pl.ds(Z, W)], v_v.at[b], rsem))
        reads.append(pltpu.make_async_copy(
            v_hbm.at[NB - 1, pl.ds(0, HKV - 1), pl.ds(Z, W)], v_v.at[NB - 1, pl.ds(0, HKV - 1)], rsem))
        if lead_rows < W:
            reads.append(pltpu.make_async_copy(
                v_hbm.at[NB - 1, HKV - 1, pl.ds(Z, W - lead_rows)],
                v_v.at[NB - 1, HKV - 1, pl.ds(0, W - lead_rows)], rsem))
        last = pltpu.make_async_copy(
            v_hbm.at[NB - 1, HKV - 1, pl.ds(SK - lead_rows, lead_rows)],
            v_v.at[NB - 1, HKV - 1, pl.ds(W - lead_rows, lead_rows)], lsem)
        for i, c in enumerate(reads):
            c.start(priority=rprio[i % len(rprio)])
        last.start(priority=rprio[len(reads) % len(rprio)])

        z_v[...] = jnp.zeros(z_v.shape, BF16)
        q_s[...] = jnp.zeros(q_s.shape, F32)
        do_s[...] = jnp.zeros(do_s.shape, F32)

        for c in reads:
            c.wait()

        nz = Z // zr

        def zero_fill(lo, hi):
            for o in (dk_hbm, dv_hbm):
                def body(i, _):
                    b = i // nz
                    r = pl.multiple_of((i - b * nz) * zr, zr)
                    pltpu.make_async_copy(z_v, o.at[b, :, pl.ds(r, zr)], wsem).start()
                lax.fori_loop(lo, hi, body, None)

        per = NB * nz // (HKV * NB + 4)
        zero_fill(0, 2 * per)
        last.wait()

        x = x_v[...].astype(F32)
        go = go_v[...].astype(F32)
        xn, rstd1 = _ln(x)
        ln2, rstd2 = _ln(xn)
        xn_b = xn.astype(BF16)
        ln2_b = ln2.astype(BF16)

        def ff_fwd(j, h2):
            c = pl.ds(pl.multiple_of(j * FB, FB), FB)
            u = _mm(ln2_b, w3_v[:, c])
            u_s[j] = u
            a = 0.5 * u * (1.0 + jnp.tanh(GELU_C * (u + 0.044715 * u * u * u)))
            return h2 + _mm(a.astype(BF16), w4_v[c, :])

        bo = xn + lax.fori_loop(0, FF // FB, ff_fwd, jnp.zeros((NB, D), F32))
        sig = jax.nn.sigmoid(bo)
        g = bo * sig
        ds_b = (go * g).astype(BF16)

        def kv_head(h, carry):
            s, dxn = carry
            c = pl.ds(pl.multiple_of(h * GW, GW), GW)
            q = _mm(xn_b, wq_v[:, c])
            do = _mm(ds_b, wo_v[c, :], NT)
            for j in range(REP):
                rows = pl.ds(j, NB, stride=8)
                q_s[rows, :] = q[:, j * DH:(j + 1) * DH]
                do_s[rows, :] = do[:, j * DH:(j + 1) * DH]

            def one(b, _):
                it = h * NB + b
                zero_fill((2 + it) * per, (3 + it) * per)
                rows = pl.ds(pl.multiple_of(b * 8, 8), 8)
                qb = q_s[rows, :].astype(BF16)
                dob = do_s[rows, :].astype(BF16)
                k = k_v[b, h]
                v = v_v[b, h]
                sc = _mm(qb, k, NT) * SCALE
                e = jnp.exp(sc - jnp.max(sc, axis=-1, keepdims=True))
                p = e / jnp.sum(e, axis=-1, keepdims=True)
                dp = _mm(dob, v, NT)
                dsc = p * (dp - jnp.sum(p * dp, axis=-1, keepdims=True)) * SCALE
                p_b = p.astype(BF16)
                dsc_b = dsc.astype(BF16)
                o_s[rows, :] = _mm(p_b, v)
                dq_s[rows, :] = _mm(dsc_b, k)
                dk_v[b, h] = _mm(dsc_b, qb, TN).astype(BF16)
                dv_v[b, h] = _mm(p_b, dob, TN).astype(BF16)

            lax.fori_loop(0, NB, one, None)

            o_b = jnp.concatenate(
                [o_s[pl.ds(j, NB, stride=8), :] for j in range(REP)], axis=1).astype(BF16)
            dq_b = jnp.concatenate(
                [dq_s[pl.ds(j, NB, stride=8), :] for j in range(REP)], axis=1).astype(BF16)
            dwo_v[c, :] = _mm(o_b, ds_b, TN).astype(BF16)
            dwq_v[:, c] = _mm(xn_b, dq_b, TN).astype(BF16)
            return s + _mm(o_b, wo_v[c, :]), dxn + _mm(dq_b, wq_v[:, c], NT)

        zero = jnp.zeros((NB, D), F32)
        s, dxn = lax.fori_loop(0, HKV, kv_head, (zero, zero))
        zero_fill((2 + HKV * NB) * per, NB * nz)
        out_v[...] = (x + s * g).astype(BF16)

        dbo = go * s * (sig * (1.0 + bo * (1.0 - sig)))
        dbo_b = dbo.astype(BF16)

        def ff_bwd(j, dln2):
            c = pl.ds(pl.multiple_of(j * FB, FB), FB)
            u = u_s[j]
            t = jnp.tanh(GELU_C * (u + 0.044715 * u * u * u))
            a = 0.5 * u * (1.0 + t)
            dgelu = 0.5 * (1.0 + t) + 0.5 * u * (1.0 - t * t) * GELU_C * (1.0 + 3 * 0.044715 * u * u)
            du_b = (_mm(dbo_b, w4_v[c, :], NT) * dgelu).astype(BF16)
            dw4_v[c, :] = _mm(a.astype(BF16), dbo_b, TN).astype(BF16)
            dw3_v[:, c] = _mm(ln2_b, du_b, TN).astype(BF16)
            return dln2 + _mm(du_b, w3_v[:, c], NT)

        dln2 = lax.fori_loop(0, FF // FB, ff_bwd, zero)
        dxn = dxn + dbo + _ln_bwd(dln2, ln2, rstd2)
        dx_v[...] = (go + _ln_bwd(dxn, xn, rstd1)).astype(BF16)

        small = [pltpu.make_async_copy(s_, d_, wsem) for s_, d_ in (
            (out_v, out_hbm), (dx_v, dx_hbm), (dwq_v, dwq_hbm), (dwo_v, dwo_hbm),
            (dw3_v, dw3_hbm), (dw4_v, dw4_hbm))]
        for c in small:
            c.start()
        nw = W // wr
        for src, o in ((dk_v, dk_hbm), (dv_v, dv_hbm)):
            def body(i, _):
                b = i // nw
                r = pl.multiple_of((i - b * nw) * wr, wr)
                pltpu.make_async_copy(
                    src.at[b, :, pl.ds(r, wr)], o.at[b, :, pl.ds(Z + r, wr)], wsem).start()
            lax.fori_loop(0, NB * nw, body, None)

        for c in small:
            c.wait()
        pltpu.make_async_copy(dk_hbm, dk_hbm, wsem).wait()
        pltpu.make_async_copy(dv_hbm, dv_hbm, wsem).wait()

    def fn(A_x, A_k_cache, A_v_cache, A_wq, A_wo, B_x, B_w1, B_w2, B_w3, B_w4, grad_out):
        hbm = pl.BlockSpec(memory_space=pltpu.HBM)
        sds = jax.ShapeDtypeStruct
        outs = pl.pallas_call(
            kernel,
            in_specs=[hbm] * 8,
            out_specs=[hbm] * 8,
            out_shape=[
                sds((NB, D), BF16), sds((NB, D), BF16),
                sds(A_k_cache.shape, BF16), sds(A_v_cache.shape, BF16),
                sds(A_wq.shape, BF16), sds(A_wo.shape, BF16),
                sds(B_w3.shape, BF16), sds(B_w4.shape, BF16),
            ],
            scratch_shapes=[
                pltpu.VMEM((NB, D), BF16), pltpu.VMEM((NB, D), BF16),
                pltpu.VMEM((NB, HKV, W, DH), BF16), pltpu.VMEM((NB, HKV, W, DH), BF16),
                pltpu.VMEM((D, HQ * DH), BF16), pltpu.VMEM((HQ * DH, D), BF16),
                pltpu.VMEM((D, FF), BF16), pltpu.VMEM((FF, D), BF16),
                pltpu.VMEM((NB, D), BF16), pltpu.VMEM((NB, D), BF16),
                pltpu.VMEM((NB, HKV, W, DH), BF16), pltpu.VMEM((NB, HKV, W, DH), BF16),
                pltpu.VMEM((D, HQ * DH), BF16), pltpu.VMEM((HQ * DH, D), BF16),
                pltpu.VMEM((D, FF), BF16), pltpu.VMEM((FF, D), BF16),
                pltpu.VMEM((HKV, zr, DH), BF16),
                pltpu.VMEM((FF // FB, NB, FB), F32),
                pltpu.VMEM((NB * 8, DH), F32), pltpu.VMEM((NB * 8, DH), F32),
                pltpu.VMEM((NB * 8, DH), F32), pltpu.VMEM((NB * 8, DH), F32),
                pltpu.SemaphoreType.DMA((3,)),
            ],
            compiler_params=pltpu.CompilerParams(vmem_limit_bytes=110 * 2**20),
        )(A_x.reshape(NB, D), A_k_cache, A_v_cache, A_wq, A_wo, B_w3, B_w4,
          grad_out.reshape(NB, D))
        return (outs[0].reshape(A_x.shape), outs[1].reshape(A_x.shape), *outs[2:])

    return fn


_impl = make()


@jax.jit
def pallas_recurrent_scan__sliding_block_cached__mixer_s_mlp__decode_kernel(
    A_x, A_k_cache, A_v_cache, A_wq, A_wo, B_x, B_w1, B_w2, B_w3, B_w4, grad_out,
):
    return _impl(A_x, A_k_cache, A_v_cache, A_wq, A_wo, B_x, B_w1, B_w2, B_w3, B_w4, grad_out)
```

```python
import math

import jax
import jax.numpy as jnp
from jax import lax
from jax.experimental import pallas as pl
from jax.experimental.pallas import tpu as pltpu

F32 = jnp.float32
BF16 = jnp.bfloat16

NB, D = 4, 512
HQ, HKV, DH = 32, 8, 128
REP = HQ // HKV
SK = 8192
W = min(4096, max(256, SK // 4))
Z = SK - W
FF = 1792
FB = 128
NF = FF // FB
GW = REP * DH
EPS = 1e-5
SCALE = DH ** -0.5
GELU_C = math.sqrt(2.0 / math.pi)
GELU_A = 0.044715

NT = (((1,), (1,)), ((), ()))
TN = (((0,), (0,)), ((), ()))

NS, NC = 8, 4
ROWS = 16


def _ln(x):
    c = x - jnp.mean(x, axis=-1, keepdims=True)
    rstd = lax.rsqrt(jnp.mean(c * c, axis=-1, keepdims=True) + EPS)
    return c * rstd, rstd


def _ln_bwd(dy, y, rstd):
    return rstd * (dy - jnp.mean(dy, axis=-1, keepdims=True)
                   - y * jnp.mean(dy * y, axis=-1, keepdims=True))


def _mm(a, b, dims=(((1,), (0,)), ((), ()))):
    return lax.dot_general(a, b, dims, preferred_element_type=F32)


def _ds(start, size):
    return pl.ds(pl.multiple_of(start, size), size)


def _row_block(ref, i, n):
    per_group = ref.shape[1] // n
    g = lax.div(i, per_group)
    return ref.at[g, _ds((i - g * per_group) * n, n)]


def make(groups=(((0, 0, 5),), ((1, 2, 6),), ((0, 5, 3), (1, 0, 2))), lead=14, batch=32, unroll=8,
         compute=True, nosc=False, tail="0123",
         rg=(4, 4, 8, 2), rp=((8, 512), (8, 512), (8, 256), (16, 512)),
         wg=(4, 4, 2, 2), wp=((8, 256),) * 4, kvoff=0):
    gmax = max(n for grp in groups for _, _, n in grp)

    def kernel(x_hbm, k_hbm, v_hbm, wq_hbm, wo_hbm, w3_hbm, w4_hbm, go_hbm,
               out_hbm, dx_hbm, dk_hbm, dv_hbm, dwq_hbm, dwo_hbm, dw3_hbm, dw4_hbm,
               x_v, go_v, k_v, v_v, wq_v, wo_v, w3_v, w4_v,
               out_v, dx_v, dk_v, dv_v, dwq_v, dwo_v, dw3_v, dw4_v,
               z_v, u_s, q_s, do_s, o_s, dq_s, sems):
        read_sem, last_sem, write_sem = sems.at[0], sems.at[1], sems.at[2]

        def wait(ref, sem):
            pltpu.make_async_copy(ref, ref, sem).wait()

        def copy_matrices(a, b, sem, queues):
            (n,) = {src.shape[1] // r * (src.shape[2] // c) for src, _, (r, c) in (a, b)}

            def body(i, _):
                for (src, dst, (r, c)), queue in zip((a, b), queues):
                    nc = src.shape[2] // c
                    j = lax.div(i, nc)
                    idx = (slice(None), _ds(j * r, r), _ds((i - j * nc) * c, c))
                    pltpu.make_async_copy(src.at[idx], dst.at[idx], sem).start(priority=queue)
            lax.fori_loop(0, n, body, None)

        def read_windows(lo, hi, sem):
            def body(i, _):
                b = lax.div(i, W // ROWS)
                r = (i - b * (W // ROWS)) * ROWS
                for queue, (src, dst) in enumerate(((k_hbm, k_v), (v_hbm, v_v))):
                    if queue and kvoff:
                        r = lax.rem(r + kvoff, W)
                    pltpu.make_async_copy(
                        src.at[b, :, _ds(Z + r, ROWS)], dst.at[b, :, _ds(r, ROWS)],
                        sem).start(priority=queue)
            lax.fori_loop(lo, hi, body, None)

        copy_matrices((wq_hbm, wq_v, rp[0]), (wo_hbm, wo_v, rp[1]), read_sem, (0, 1))
        pltpu.make_async_copy(x_hbm, x_v, read_sem).start(priority=0)
        pltpu.make_async_copy(go_hbm, go_v, read_sem).start(priority=1)
        copy_matrices((w3_hbm, w3_v, rp[2]), (w4_hbm, w4_v, rp[3]), read_sem, (0, 1))
        read_windows(0, NB * W // ROWS - lead, read_sem)
        read_windows(NB * W // ROWS - lead, NB * W // ROWS, last_sem)

        z_v[...] = jnp.zeros(z_v.shape, BF16)
        q_s[...] = jnp.zeros(q_s.shape, F32)
        do_s[...] = jnp.zeros(do_s.shape, F32)

        for ref in (x_v, go_v, wq_v, wo_v, w3_v, w4_v):
            wait(ref, read_sem)
        for ref in (k_v, v_v):
            wait(ref.at[pl.ds(0, NB - 1)], read_sem)
            wait(ref.at[NB - 1, :, pl.ds(0, W - lead * ROWS)], read_sem)

        cache_grads = (dk_hbm, dv_hbm)
        staged = (dk_v, dv_v)
        zero_batches = Z // (ROWS * batch)
        window_batches = W // (ROWS * batch)

        def write_batch(group, i, zeros):
            per_column = zero_batches if zeros else window_batches
            c = lax.div(i, per_column)
            r0 = (i - c * per_column) * (ROWS * batch)

            def body(j, _):
                for u in range(unroll):
                    r = r0 + (j * unroll + u) * ROWS
                    for t, s0, n in group:
                        if zeros:
                            src = z_v.at[pl.ds(0, n)]
                        else:
                            src = staged[t].at[pl.ds(s0, n), c, _ds(r, ROWS)]
                        dst = cache_grads[t].at[pl.ds(s0, n), c, _ds(r if zeros else Z + r, ROWS)]
                        pltpu.make_async_copy(src, dst, write_sem).start()
            lax.fori_loop(0, batch // unroll, body, None)

        def write_batches(group, lo, hi, zeros):
            lax.fori_loop(lo, hi, lambda i, _: write_batch(group, i, zeros), None)

        nzero = NC * zero_batches

        def feed(i):
            pl.when(i < nzero)(lambda: write_batch(groups[0], i, True))
            pl.when(i >= nzero)(lambda: write_batch(groups[1], i - nzero, True))

        per_head = 2 * NB + 3
        first_head = 2 * nzero - HKV * per_head
        ahead = first_head - NF // 2 + 1
        assert ahead >= 2
        write_batches(groups[0], 0, ahead, True)

        def wait_last():
            for ref in (k_v, v_v):
                wait(ref.at[NB - 1, :, pl.ds(W - lead * ROWS, lead * ROWS)], last_sem)

        if compute:
            x = x_v[...].astype(F32)
            go = go_v[...].astype(F32)
            xn, rstd1 = _ln(x)
            ln2, rstd2 = _ln(xn)
            xn_b = xn.astype(BF16)
            ln2_b = ln2.astype(BF16)

            def ff_fwd(j, h2):
                pl.when(jnp.logical_and(j > 0, lax.rem(j, 2) == 0))(
                    lambda: write_batch(groups[0], ahead - 1 + lax.div(j, 2), True))
                u = _mm(ln2_b, w3_v[:, :, _ds(j * FB, FB)].reshape(D, FB))
                u_s[j] = u
                a = 0.5 * u * (1.0 + jnp.tanh(GELU_C * (u + GELU_A * u * u * u)))
                return h2 + _mm(a.astype(BF16), _row_block(w4_v, j, FB)[...])

            zero = jnp.zeros((NB, D), F32)
            bo = xn + lax.fori_loop(0, NF, ff_fwd, zero)
            sig = jax.nn.sigmoid(bo)
            g = bo * sig
            ds_b = (go * g).astype(BF16)
            wait_last()

            def kv_head(h, carry):
                s, dxn = carry
                i0 = first_head + h * per_head
                feed(i0)
                cols = _ds(h * GW, GW)
                wo_h = _row_block(wo_v, h, GW)
                q = _mm(xn_b, wq_v[:, :, cols].reshape(D, GW))
                do = _mm(ds_b, wo_h[...], NT)
                for j in range(REP):
                    rows = pl.ds(j, NB, stride=8)
                    q_s[rows, :] = q[:, j * DH:(j + 1) * DH]
                    do_s[rows, :] = do[:, j * DH:(j + 1) * DH]

                def sample(b, _):
                    feed(i0 + 1 + 2 * b)
                    rows = _ds(b * 8, 8)
                    q_b = q_s[rows, :].astype(BF16)
                    do_b = do_s[rows, :].astype(BF16)
                    sc = _mm(q_b, k_v[b, h], NT) * SCALE
                    e = jnp.exp(sc - jnp.max(sc, axis=-1, keepdims=True))
                    p = e / jnp.sum(e, axis=-1, keepdims=True)
                    dp = _mm(do_b, v_v[b, h], NT)
                    dsc = p * (dp - jnp.sum(p * dp, axis=-1, keepdims=True)) * SCALE
                    p_b = p.astype(BF16)
                    dsc_b = dsc.astype(BF16)
                    o_s[rows, :] = _mm(p_b, v_v[b, h])
                    dq_s[rows, :] = _mm(dsc_b, k_v[b, h])
                    feed(i0 + 2 + 2 * b)
                    plane = b * HKV + h
                    ps = lax.div(plane, NC)
                    dk_v[ps, plane - ps * NC] = _mm(dsc_b, q_b, TN).astype(BF16)
                    dv_v[ps, plane - ps * NC] = _mm(p_b, do_b, TN).astype(BF16)

                lax.fori_loop(0, NB, sample, None)

                def heads(ref):
                    return jnp.concatenate(
                        [ref[pl.ds(j, NB, stride=8), :] for j in range(REP)], axis=1).astype(BF16)

                feed(i0 + 1 + 2 * NB)
                o_b = heads(o_s)
                _row_block(dwo_v, h, GW)[...] = _mm(o_b, ds_b, TN).astype(BF16)
                s = s + _mm(o_b, wo_h[...])
                feed(i0 + 2 + 2 * NB)
                dq_b = heads(dq_s)
                dwq_v[:, :, cols] = _mm(xn_b, dq_b, TN).astype(BF16).reshape(wg[0], -1, GW)
                return s, dxn + _mm(dq_b, wq_v[:, :, cols].reshape(D, GW), NT)

            s, dxn = lax.fori_loop(0, HKV, kv_head, (zero, zero))
            write_batch(groups[0], 0, False)
            out_v[...] = (x + s * g).astype(BF16)

            dbo = go * s * (sig * (1.0 + bo * (1.0 - sig)))
            dbo_b = dbo.astype(BF16)

            def ff_bwd(j, dln2):
                write_batch(groups[0], j + 1, False)
                cols = _ds(j * FB, FB)
                u = u_s[j]
                t = jnp.tanh(GELU_C * (u + GELU_A * u * u * u))
                a = 0.5 * u * (1.0 + t)
                dgelu = (0.5 * (1.0 + t)
                         + 0.5 * u * (1.0 - t * t) * GELU_C * (1.0 + 3 * GELU_A * u * u))
                du_b = (_mm(dbo_b, _row_block(w4_v, j, FB)[...], NT) * dgelu).astype(BF16)
                _row_block(dw4_v, j, FB)[...] = _mm(a.astype(BF16), dbo_b, TN).astype(BF16)
                dw3_v[:, :, cols] = _mm(ln2_b, du_b, TN).astype(BF16).reshape(wg[2], -1, FB)
                return dln2 + _mm(du_b, w3_v[:, :, cols].reshape(D, FB), NT)

            dln2 = lax.fori_loop(0, NF, ff_bwd, zero)
            write_batches(groups[0], NF + 1, NC * window_batches, False)
            dxn = dxn + dbo + _ln_bwd(dln2, ln2, rstd2)
            dx_v[...] = (go + _ln_bwd(dxn, xn, rstd1)).astype(BF16)
        else:
            lax.fori_loop(ahead, 2 * nzero, lambda i, _: feed(i), None)
            wait_last()
            write_batches(groups[0], 0, NC * window_batches, False)

        def weights():
            pltpu.make_async_copy(out_v, out_hbm, write_sem).start()
            pltpu.make_async_copy(dx_v, dx_hbm, write_sem).start()
            copy_matrices((dwq_v, dwq_hbm, wp[0]), (dwo_v, dwo_hbm, wp[1]), write_sem, (0, 0))
            copy_matrices((dw3_v, dw3_hbm, wp[2]), (dw4_v, dw4_hbm, wp[3]), write_sem, (0, 0))

        rest = (lambda: write_batches(groups[1], 0, NC * window_batches, False),
                lambda: write_batches(groups[2], 0, nzero, True),
                lambda: write_batches(groups[2], 0, NC * window_batches, False),
                weights)
        for ch in tail:
            rest[int(ch)]()

        for ref in (out_hbm, dx_hbm, dwq_hbm, dwo_hbm, dw3_hbm, dw4_hbm, dk_hbm, dv_hbm):
            wait(ref, write_sem)

    def fn(A_x, A_k_cache, A_v_cache, A_wq, A_wo, B_x, B_w1, B_w2, B_w3, B_w4, grad_out):
        hbm = pl.BlockSpec(memory_space=pltpu.HBM)
        sds = jax.ShapeDtypeStruct
        mats = ((D, HQ * DH), (HQ * DH, D), (D, FF), (FF, D))
        rshape = [(g, r // g, c) for g, (r, c) in zip(rg, mats)]
        wshape = [(g, r // g, c) for g, (r, c) in zip(wg, mats)]
        outs = pl.pallas_call(
            kernel,
            in_specs=[hbm] * 8,
            out_specs=[hbm] * 8,
            out_shape=[
                sds((NB, D), BF16), sds((NB, D), BF16),
                sds((NS, NC, SK, DH), BF16), sds((NS, NC, SK, DH), BF16),
                *[sds(s, BF16) for s in wshape],
            ],
            scratch_shapes=[
                pltpu.VMEM((NB, D), BF16), pltpu.VMEM((NB, D), BF16),
                pltpu.VMEM((NB, HKV, W, DH), BF16), pltpu.VMEM((NB, HKV, W, DH), BF16),
                *[pltpu.VMEM(s, BF16) for s in rshape],
                pltpu.VMEM((NB, D), BF16), pltpu.VMEM((NB, D), BF16),
                pltpu.VMEM((NS, NC, W, DH), BF16), pltpu.VMEM((NS, NC, W, DH), BF16),
                *[pltpu.VMEM(s, BF16) for s in wshape],
                pltpu.VMEM((gmax, ROWS, DH), BF16),
                pltpu.VMEM((NF, NB, FB), F32),
                pltpu.VMEM((NB * 8, DH), F32), pltpu.VMEM((NB * 8, DH), F32),
                pltpu.VMEM((NB * 8, DH), F32), pltpu.VMEM((NB * 8, DH), F32),
                pltpu.SemaphoreType.DMA((3,)),
            ],
            compiler_params=pltpu.CompilerParams(
                vmem_limit_bytes=110 * 2**20, disable_bounds_checks=True,
                disable_semaphore_checks=nosc),
        )(A_x.reshape(NB, D), A_k_cache, A_v_cache,
          *[w.reshape(s) for w, s in zip((A_wq, A_wo, B_w3, B_w4), rshape)],
          grad_out.reshape(NB, D))
        shapes = [a.shape for a in (A_x, A_x, A_k_cache, A_v_cache, A_wq, A_wo, B_w3, B_w4)]
        return tuple(o.reshape(s) for o, s in zip(outs, shapes))

    return fn


_impl = make(kvoff=64)


@jax.jit
def pallas_recurrent_scan__sliding_block_cached__mixer_s_mlp__decode_kernel(
    A_x, A_k_cache, A_v_cache, A_wq, A_wo, B_x, B_w1, B_w2, B_w3, B_w4, grad_out,
):
    return _impl(A_x, A_k_cache, A_v_cache, A_wq, A_wo, B_x, B_w1, B_w2, B_w3, B_w4, grad_out)
```

```python
import math

import jax
import jax.numpy as jnp
from jax import lax
from jax.experimental import pallas as pl
from jax.experimental.pallas import tpu as pltpu

F32 = jnp.float32
BF16 = jnp.bfloat16

NB, D = 4, 512
HQ, HKV, DH = 32, 8, 128
REP = HQ // HKV
GW = REP * DH
SK = 8192
W = min(4096, max(256, SK // 4))
Z = SK - W
FF, FB = 1792, 128
NF = FF // FB
EPS = 1e-5
SCALE = DH ** -0.5
GELU_C = math.sqrt(2.0 / math.pi)
GELU_A = 0.044715

NT = (((1,), (1,)), ((), ()))
TN = (((0,), (0,)), ((), ()))

MATRICES = ((D, HQ * DH), (HQ * DH, D), (D, FF), (FF, D))
READ_GROUPS = (8, 8, 8, 2)
READ_PIECES = ((8, 256), (8, 256), (8, 256), (16, 512))
WRITE_GROUPS = (4, 4, 2, 2)
WRITE_PIECE = (8, 256)

NS, NC = 8, 4
STREAMS = (((0, 0, 5),), ((1, 2, 6),), ((0, 5, 3), (1, 0, 2)))
ROWS = 16
BATCH, UNROLL = 32, 8
ZERO_BATCHES = NC * Z // (ROWS * BATCH)
WINDOW_BATCHES = NC * W // (ROWS * BATCH)
V_SHIFT = 64
LEAD = 7

FEEDS_PER_HEAD = 2 * NB + 3
FIRST_HEAD_FEED = 2 * ZERO_BATCHES - HKV * FEEDS_PER_HEAD
FF_FEED_EVERY = 4
FEEDS_AHEAD = FIRST_HEAD_FEED - (NF - 1) // FF_FEED_EVERY


def _layernorm(x):
    c = x - jnp.mean(x, axis=-1, keepdims=True)
    rstd = lax.rsqrt(jnp.mean(c * c, axis=-1, keepdims=True) + EPS)
    return c * rstd, rstd


def _layernorm_bwd(dy, y, rstd):
    return rstd * (dy - jnp.mean(dy, axis=-1, keepdims=True)
                   - y * jnp.mean(dy * y, axis=-1, keepdims=True))


def _gelu_tanh(u):
    return jnp.tanh(GELU_C * (u + GELU_A * u * u * u))


def _mm(a, b, dims=(((1,), (0,)), ((), ()))):
    return lax.dot_general(a, b, dims, preferred_element_type=F32)


def _ds(start, size):
    return pl.ds(pl.multiple_of(start, size), size)


def _row_block(ref, i, n):
    per_group = ref.shape[1] // n
    g = lax.div(i, per_group)
    return ref.at[g, _ds((i - g * per_group) * n, n)]


def _wait(ref, sem):
    pltpu.make_async_copy(ref, ref, sem).wait()


def _copy_matrices(pair, sem, queues):
    counts = [src.shape[1] // r * (src.shape[2] // c) for src, _, (r, c) in pair]
    assert counts[0] == counts[1]

    def body(i, _):
        for (src, dst, (r, c)), queue in zip(pair, queues):
            per_row = src.shape[2] // c
            j = lax.div(i, per_row)
            piece = (slice(None), _ds(j * r, r), _ds((i - j * per_row) * c, c))
            pltpu.make_async_copy(src.at[piece], dst.at[piece], sem).start(priority=queue)

    lax.fori_loop(0, counts[0], body, None)


def _kernel(x_hbm, k_hbm, v_hbm, wq_hbm, wo_hbm, w3_hbm, w4_hbm, go_hbm,
            out_hbm, dx_hbm, dk_hbm, dv_hbm, dwq_hbm, dwo_hbm, dw3_hbm, dw4_hbm,
            x_v, go_v, k_v, v_v, wq_v, wo_v, w3_v, w4_v,
            out_v, dx_v, dk_v, dv_v, dwq_v, dwo_v, dw3_v, dw4_v,
            zero_v, u_s, q_s, do_s, o_s, dq_s, sems):
    read_sem, write_sem = sems.at[0], sems.at[1]

    pltpu.make_async_copy(x_hbm, x_v, read_sem).start(priority=0)
    pltpu.make_async_copy(go_hbm, go_v, read_sem).start(priority=1)
    _copy_matrices(((w3_hbm, w3_v, READ_PIECES[2]), (w4_hbm, w4_v, READ_PIECES[3])),
                   read_sem, (0, 1))

    def read_windows(i, _):
        b = lax.div(i, W // ROWS)
        r = (i - b * (W // ROWS)) * ROWS
        for queue, (src, dst, row) in enumerate(
                ((k_hbm, k_v, r), (v_hbm, v_v, lax.rem(r + V_SHIFT, W)))):
            pltpu.make_async_copy(src.at[b, :, _ds(Z + row, ROWS)], dst.at[b, :, _ds(row, ROWS)],
                                  read_sem).start(priority=queue)

    lax.fori_loop(0, NB * W // ROWS, read_windows, None)
    _copy_matrices(((wq_hbm, wq_v, READ_PIECES[0]), (wo_hbm, wo_v, READ_PIECES[1])),
                   read_sem, (0, 1))

    zero_v[...] = jnp.zeros(zero_v.shape, BF16)
    q_s[...] = jnp.zeros(q_s.shape, F32)
    do_s[...] = jnp.zeros(do_s.shape, F32)

    for ref in (x_v, go_v, wq_v, wo_v, w3_v, w4_v):
        _wait(ref, read_sem)
    for ref in (k_v, v_v):
        _wait(ref.at[pl.ds(0, NB - 1)], read_sem)
        _wait(ref.at[NB - 1, :, pl.ds(0, W - LEAD * ROWS)], read_sem)

    def write_batch(streams, i, zeros):
        per_column = (ZERO_BATCHES if zeros else WINDOW_BATCHES) // NC
        col = lax.div(i, per_column)
        first = (i - col * per_column) * (ROWS * BATCH)

        def body(j, _):
            for u in range(UNROLL):
                row = first + (j * UNROLL + u) * ROWS
                for which, s0, n in streams:
                    planes = pl.ds(s0, n)
                    if zeros:
                        src = zero_v.at[pl.ds(0, n)]
                    else:
                        src = (dk_v, dv_v)[which].at[planes, col, _ds(row, ROWS)]
                    dst = (dk_hbm, dv_hbm)[which].at[
                        planes, col, _ds(row if zeros else Z + row, ROWS)]
                    pltpu.make_async_copy(src, dst, write_sem).start()

        lax.fori_loop(0, BATCH // UNROLL, body, None)

    def write_batches(streams, lo, hi, zeros):
        lax.fori_loop(lo, hi, lambda i, _: write_batch(streams, i, zeros), None)

    def feed(i):
        pl.when(i < ZERO_BATCHES)(lambda: write_batch(STREAMS[0], i, True))
        pl.when(i >= ZERO_BATCHES)(lambda: write_batch(STREAMS[1], i - ZERO_BATCHES, True))

    write_batches(STREAMS[0], 0, FEEDS_AHEAD, True)
    for ref in (k_v, v_v):
        _wait(ref.at[NB - 1, :, pl.ds(W - LEAD * ROWS, LEAD * ROWS)], read_sem)

    x = x_v[...].astype(F32)
    go = go_v[...].astype(F32)
    xn, rstd1 = _layernorm(x)
    ln2, rstd2 = _layernorm(xn)
    xn_b = xn.astype(BF16)
    ln2_b = ln2.astype(BF16)
    zero = jnp.zeros((NB, D), F32)

    def ff_fwd(j, h2):
        pl.when(jnp.logical_and(j > 0, lax.rem(j, FF_FEED_EVERY) == 0))(
            lambda: write_batch(STREAMS[0], FEEDS_AHEAD - 1 + lax.div(j, FF_FEED_EVERY), True))
        u = _mm(ln2_b, w3_v[:, :, _ds(j * FB, FB)].reshape(D, FB))
        u_s[j] = u
        a = 0.5 * u * (1.0 + _gelu_tanh(u))
        return h2 + _mm(a.astype(BF16), _row_block(w4_v, j, FB)[...])

    bo = xn + lax.fori_loop(0, NF, ff_fwd, zero)
    sig = jax.nn.sigmoid(bo)
    g = bo * sig
    ds_b = (go * g).astype(BF16)

    def kv_head(h, carry):
        s, dxn = carry
        slot = FIRST_HEAD_FEED + h * FEEDS_PER_HEAD
        feed(slot)
        cols = _ds(h * GW, GW)
        wo_h = _row_block(wo_v, h, GW)
        q = _mm(xn_b, wq_v[:, :, cols].reshape(D, GW))
        do = _mm(ds_b, wo_h[...], NT)
        for j in range(REP):
            rows = pl.ds(j, NB, stride=8)
            q_s[rows, :] = q[:, j * DH:(j + 1) * DH]
            do_s[rows, :] = do[:, j * DH:(j + 1) * DH]

        def sample(b, _):
            feed(slot + 1 + 2 * b)
            rows = _ds(b * 8, 8)
            q_b = q_s[rows, :].astype(BF16)
            do_b = do_s[rows, :].astype(BF16)
            scores = _mm(q_b, k_v[b, h], NT) * SCALE
            e = jnp.exp(scores - jnp.max(scores, axis=-1, keepdims=True))
            p = e / jnp.sum(e, axis=-1, keepdims=True)
            dp = _mm(do_b, v_v[b, h], NT)
            dscores = p * (dp - jnp.sum(p * dp, axis=-1, keepdims=True)) * SCALE
            p_b = p.astype(BF16)
            dscores_b = dscores.astype(BF16)
            o_s[rows, :] = _mm(p_b, v_v[b, h])
            dq_s[rows, :] = _mm(dscores_b, k_v[b, h])
            feed(slot + 2 + 2 * b)
            plane = b * HKV + h
            row = lax.div(plane, NC)
            dk_v[row, plane - row * NC] = _mm(dscores_b, q_b, TN).astype(BF16)
            dv_v[row, plane - row * NC] = _mm(p_b, do_b, TN).astype(BF16)

        lax.fori_loop(0, NB, sample, None)

        def heads(ref):
            return jnp.concatenate(
                [ref[pl.ds(j, NB, stride=8), :] for j in range(REP)], axis=1).astype(BF16)

        feed(slot + 1 + 2 * NB)
        o_b = heads(o_s)
        _row_block(dwo_v, h, GW)[...] = _mm(o_b, ds_b, TN).astype(BF16)
        s = s + _mm(o_b, wo_h[...])
        feed(slot + 2 + 2 * NB)
        dq_b = heads(dq_s)
        dwq_v[:, :, cols] = _mm(xn_b, dq_b, TN).astype(BF16).reshape(dwq_v.shape[0], -1, GW)
        return s, dxn + _mm(dq_b, wq_v[:, :, cols].reshape(D, GW), NT)

    s, dxn = lax.fori_loop(0, HKV, kv_head, (zero, zero))
    write_batch(STREAMS[0], 0, False)
    out_v[...] = (x + s * g).astype(BF16)

    dbo = go * s * (sig * (1.0 + bo * (1.0 - sig)))
    dbo_b = dbo.astype(BF16)

    def ff_bwd(j, dln2):
        write_batch(STREAMS[0], j + 1, False)
        cols = _ds(j * FB, FB)
        u = u_s[j]
        t = _gelu_tanh(u)
        a = 0.5 * u * (1.0 + t)
        dgelu = 0.5 * (1.0 + t) + 0.5 * u * (1.0 - t * t) * GELU_C * (1.0 + 3.0 * GELU_A * u * u)
        du_b = (_mm(dbo_b, _row_block(w4_v, j, FB)[...], NT) * dgelu).astype(BF16)
        _row_block(dw4_v, j, FB)[...] = _mm(a.astype(BF16), dbo_b, TN).astype(BF16)
        dw3_v[:, :, cols] = _mm(ln2_b, du_b, TN).astype(BF16).reshape(dw3_v.shape[0], -1, FB)
        return dln2 + _mm(du_b, w3_v[:, :, cols].reshape(D, FB), NT)

    dln2 = lax.fori_loop(0, NF, ff_bwd, zero)
    write_batches(STREAMS[0], NF + 1, WINDOW_BATCHES, False)
    dxn = dxn + dbo + _layernorm_bwd(dln2, ln2, rstd2)
    dx_v[...] = (go + _layernorm_bwd(dxn, xn, rstd1)).astype(BF16)

    write_batches(STREAMS[1], 0, WINDOW_BATCHES, False)
    write_batches(STREAMS[2], 0, ZERO_BATCHES, True)
    write_batches(STREAMS[2], 0, WINDOW_BATCHES, False)
    pltpu.make_async_copy(out_v, out_hbm, write_sem).start()
    pltpu.make_async_copy(dx_v, dx_hbm, write_sem).start()
    _copy_matrices(((dwq_v, dwq_hbm, WRITE_PIECE), (dwo_v, dwo_hbm, WRITE_PIECE)),
                   write_sem, (0, 0))
    _copy_matrices(((dw3_v, dw3_hbm, WRITE_PIECE), (dw4_v, dw4_hbm, WRITE_PIECE)),
                   write_sem, (0, 0))

    for ref in (out_hbm, dx_hbm, dwq_hbm, dwo_hbm, dw3_hbm, dw4_hbm, dk_hbm, dv_hbm):
        _wait(ref, write_sem)


@jax.jit
def pallas_recurrent_scan__sliding_block_cached__mixer_s_mlp__decode_kernel(
    A_x: jax.Array,
    A_k_cache: jax.Array,
    A_v_cache: jax.Array,
    A_wq: jax.Array,
    A_wo: jax.Array,
    B_x: jax.Array,
    B_w1: jax.Array,
    B_w2: jax.Array,
    B_w3: jax.Array,
    B_w4: jax.Array,
    grad_out: jax.Array,
):
    assert A_x.shape == (NB, 1, D) and A_k_cache.shape == (NB, HKV, SK, DH)
    read_shapes = [(g, r // g, c) for g, (r, c) in zip(READ_GROUPS, MATRICES)]
    write_shapes = [(g, r // g, c) for g, (r, c) in zip(WRITE_GROUPS, MATRICES)]
    hbm = pl.BlockSpec(memory_space=pltpu.HBM)

    def vmem(shapes, dtype=BF16):
        return [pltpu.VMEM(shape, dtype) for shape in shapes]

    outs = pl.pallas_call(
        _kernel,
        in_specs=[hbm] * 8,
        out_specs=[hbm] * 8,
        out_shape=[
            jax.ShapeDtypeStruct(shape, BF16)
            for shape in [(NB, D)] * 2 + [(NS, NC, SK, DH)] * 2 + write_shapes
        ],
        scratch_shapes=[
            *vmem([(NB, D)] * 2 + [(NB, HKV, W, DH)] * 2 + read_shapes),
            *vmem([(NB, D)] * 2 + [(NS, NC, W, DH)] * 2 + write_shapes),
            *vmem([(max(n for streams in STREAMS for _, _, n in streams), ROWS, DH)]),
            *vmem([(NF, NB, FB)] + [(NB * 8, DH)] * 4, F32),
            pltpu.SemaphoreType.DMA((2,)),
        ],
        compiler_params=pltpu.CompilerParams(
            vmem_limit_bytes=110 * 2**20, disable_bounds_checks=True),
    )(
        A_x.reshape(NB, D), A_k_cache, A_v_cache,
        *[w.reshape(shape) for w, shape in zip((A_wq, A_wo, B_w3, B_w4), read_shapes)],
        grad_out.reshape(NB, D),
    )
    like = (A_x, A_x, A_k_cache, A_v_cache, A_wq, A_wo, B_w3, B_w4)
    return tuple(o.reshape(a.shape) for o, a in zip(outs, like))
```

```python
import math

import jax
import jax.numpy as jnp
from jax import lax
from jax.experimental import pallas as pl
from jax.experimental.pallas import tpu as pltpu

F32 = jnp.float32
BF16 = jnp.bfloat16

NB, D = 4, 512
HQ, HKV, DH = 32, 8, 128
REP = HQ // HKV
GW = REP * DH
SK = 8192
W = min(4096, max(256, SK // 4))
Z = SK - W
FF, FB = 1792, 128
NF = FF // FB
EPS = 1e-5
SCALE = DH ** -0.5
GELU_C = math.sqrt(2.0 / math.pi)
GELU_A = 0.044715

NT = (((1,), (1,)), ((), ()))
TN = (((0,), (0,)), ((), ()))

MATRICES = ((D, HQ * DH), (HQ * DH, D), (D, FF), (FF, D))
READ_GROUPS = (8, 8, 8, 2)
READ_PIECES = ((8, 256), (8, 256), (8, 256), (16, 512))
WRITE_GROUPS = (4, 4, 2, 2)
WRITE_PIECE = (8, 256)

NS, NC = 8, 4
STREAMS = (((0, 3, 5),), ((1, 0, 6),), ((0, 0, 3), (1, 6, 2)))
ROWS = 16
BATCH, UNROLL = 32, 8
ZERO_BATCHES = NC * Z // (ROWS * BATCH)
WINDOW_BATCHES = NC * W // (ROWS * BATCH)
V_SHIFT = 64
LEAD = 7

FEEDS_PER_HEAD = 2 * NB + 3
FIRST_HEAD_FEED = 2 * ZERO_BATCHES - HKV * FEEDS_PER_HEAD
FF_FEED_EVERY = 4
FEEDS_AHEAD = FIRST_HEAD_FEED - (NF - 1) // FF_FEED_EVERY


def _layernorm(x):
    c = x - jnp.mean(x, axis=-1, keepdims=True)
    rstd = lax.rsqrt(jnp.mean(c * c, axis=-1, keepdims=True) + EPS)
    return c * rstd, rstd


def _layernorm_bwd(dy, y, rstd):
    return rstd * (dy - jnp.mean(dy, axis=-1, keepdims=True)
                   - y * jnp.mean(dy * y, axis=-1, keepdims=True))


def _gelu_tanh(u):
    return jnp.tanh(GELU_C * (u + GELU_A * u * u * u))


def _mm(a, b, dims=(((1,), (0,)), ((), ()))):
    return lax.dot_general(a, b, dims, preferred_element_type=F32)


def _ds(start, size):
    return pl.ds(pl.multiple_of(start, size), size)


def _row_block(ref, i, n):
    per_group = ref.shape[1] // n
    g = lax.div(i, per_group)
    return ref.at[g, _ds((i - g * per_group) * n, n)]


def _wait(ref, sem):
    pltpu.make_async_copy(ref, ref, sem).wait()


def _copy_matrices(pair, sem, queues):
    counts = [src.shape[1] // r * (src.shape[2] // c) for src, _, (r, c) in pair]
    assert counts[0] == counts[1]

    def body(i, _):
        for (src, dst, (r, c)), queue in zip(pair, queues):
            per_row = src.shape[2] // c
            j = lax.div(i, per_row)
            piece = (slice(None), _ds(j * r, r), _ds((i - j * per_row) * c, c))
            pltpu.make_async_copy(src.at[piece], dst.at[piece], sem).start(priority=queue)

    lax.fori_loop(0, counts[0], body, None)


def _kernel(x_hbm, k_hbm, v_hbm, wq_hbm, wo_hbm, w3_hbm, w4_hbm, go_hbm,
            out_hbm, dx_hbm, dk_hbm, dv_hbm, dwq_hbm, dwo_hbm, dw3_hbm, dw4_hbm,
            x_v, go_v, k_v, v_v, wq_v, wo_v, w3_v, w4_v,
            out_v, dx_v, dk_v, dv_v, dwq_v, dwo_v, dw3_v, dw4_v,
            zero_v, u_s, q_s, do_s, o_s, dq_s, sems):
    read_sem, write_sem = sems.at[0], sems.at[1]

    pltpu.make_async_copy(x_hbm, x_v, read_sem).start(priority=0)
    pltpu.make_async_copy(go_hbm, go_v, read_sem).start(priority=1)
    _copy_matrices(((w3_hbm, w3_v, READ_PIECES[2]), (w4_hbm, w4_v, READ_PIECES[3])),
                   read_sem, (0, 1))

    def read_windows(i, _):
        b = lax.div(i, W // ROWS)
        r = (i - b * (W // ROWS)) * ROWS
        for queue, (src, dst, row) in enumerate(
                ((k_hbm, k_v, r), (v_hbm, v_v, lax.rem(r + V_SHIFT, W)))):
            pltpu.make_async_copy(src.at[b, :, _ds(Z + row, ROWS)], dst.at[b, :, _ds(row, ROWS)],
                                  read_sem).start(priority=queue)

    lax.fori_loop(0, NB * W // ROWS, read_windows, None)
    _copy_matrices(((wq_hbm, wq_v, READ_PIECES[0]), (wo_hbm, wo_v, READ_PIECES[1])),
                   read_sem, (0, 1))

    zero_v[...] = jnp.zeros(zero_v.shape, BF16)
    q_s[...] = jnp.zeros(q_s.shape, F32)
    do_s[...] = jnp.zeros(do_s.shape, F32)

    for ref in (x_v, go_v, wq_v, wo_v, w3_v, w4_v):
        _wait(ref, read_sem)
    for ref in (k_v, v_v):
        _wait(ref.at[pl.ds(0, NB - 1)], read_sem)
        _wait(ref.at[NB - 1, :, pl.ds(0, W - LEAD * ROWS)], read_sem)

    def write_batch(streams, i, zeros):
        per_column = (ZERO_BATCHES if zeros else WINDOW_BATCHES) // NC
        col = lax.div(i, per_column)
        first = (i - col * per_column) * (ROWS * BATCH)

        def body(j, _):
            for u in range(UNROLL):
                row = first + (j * UNROLL + u) * ROWS
                for which, s0, n in streams:
                    planes = pl.ds(s0, n)
                    if zeros:
                        src = zero_v.at[pl.ds(0, n)]
                    else:
                        src = (dk_v, dv_v)[which].at[planes, col, _ds(row, ROWS)]
                    dst = (dk_hbm, dv_hbm)[which].at[
                        planes, col, _ds(row if zeros else Z + row, ROWS)]
                    pltpu.make_async_copy(src, dst, write_sem).start()

        lax.fori_loop(0, BATCH // UNROLL, body, None)

    def write_batches(streams, lo, hi, zeros):
        lax.fori_loop(lo, hi, lambda i, _: write_batch(streams, i, zeros), None)

    def feed(i):
        pl.when(i < ZERO_BATCHES)(lambda: write_batch(STREAMS[0], i, True))
        pl.when(i >= ZERO_BATCHES)(lambda: write_batch(STREAMS[1], i - ZERO_BATCHES, True))

    write_batches(STREAMS[0], 0, FEEDS_AHEAD, True)
    for ref in (k_v, v_v):
        _wait(ref.at[NB - 1, :, pl.ds(W - LEAD * ROWS, LEAD * ROWS)], read_sem)

    x = x_v[...].astype(F32)
    go = go_v[...].astype(F32)
    xn, rstd1 = _layernorm(x)
    ln2, rstd2 = _layernorm(xn)
    xn_b = xn.astype(BF16)
    ln2_b = ln2.astype(BF16)
    zero = jnp.zeros((NB, D), F32)

    def ff_fwd(j, h2):
        pl.when(jnp.logical_and(j > 0, lax.rem(j, FF_FEED_EVERY) == 0))(
            lambda: write_batch(STREAMS[0], FEEDS_AHEAD - 1 + lax.div(j, FF_FEED_EVERY), True))
        u = _mm(ln2_b, w3_v[:, :, _ds(j * FB, FB)].reshape(D, FB))
        u_s[j] = u
        a = 0.5 * u * (1.0 + _gelu_tanh(u))
        return h2 + _mm(a.astype(BF16), _row_block(w4_v, j, FB)[...])

    bo = xn + lax.fori_loop(0, NF, ff_fwd, zero)
    sig = jax.nn.sigmoid(bo)
    g = bo * sig
    ds_b = (go * g).astype(BF16)

    def kv_head(h, carry):
        s, dxn = carry
        slot = FIRST_HEAD_FEED + h * FEEDS_PER_HEAD
        feed(slot)
        cols = _ds(h * GW, GW)
        wo_h = _row_block(wo_v, h, GW)
        q = _mm(xn_b, wq_v[:, :, cols].reshape(D, GW))
        do = _mm(ds_b, wo_h[...], NT)
        for j in range(REP):
            q_s[:, j, :] = q[:, j * DH:(j + 1) * DH]
            do_s[:, j, :] = do[:, j * DH:(j + 1) * DH]

        def sample(b, _):
            feed(slot + 1 + 2 * b)
            q_b = q_s[b].astype(BF16)
            do_b = do_s[b].astype(BF16)
            scores = _mm(q_b, k_v[b, h], NT) * SCALE
            e = jnp.exp(scores - jnp.max(scores, axis=-1, keepdims=True))
            p = e / jnp.sum(e, axis=-1, keepdims=True)
            dp = _mm(do_b, v_v[b, h], NT)
            dscores = p * (dp - jnp.sum(p * dp, axis=-1, keepdims=True)) * SCALE
            p_b = p.astype(BF16)
            dscores_b = dscores.astype(BF16)
            o_s[b] = _mm(p_b, v_v[b, h])
            dq_s[b] = _mm(dscores_b, k_v[b, h])
            feed(slot + 2 + 2 * b)
            plane = b * HKV + h
            row = lax.div(plane, NC)
            dk_v[row, plane - row * NC] = _mm(dscores_b, q_b, TN).astype(BF16)
            dv_v[row, plane - row * NC] = _mm(p_b, do_b, TN).astype(BF16)

        lax.fori_loop(0, NB, sample, None)

        def heads(ref):
            return jnp.concatenate([ref[:, j, :] for j in range(REP)], axis=1).astype(BF16)

        feed(slot + 1 + 2 * NB)
        o_b = heads(o_s)
        _row_block(dwo_v, h, GW)[...] = _mm(o_b, ds_b, TN).astype(BF16)
        s = s + _mm(o_b, wo_h[...])
        feed(slot + 2 + 2 * NB)
        dq_b = heads(dq_s)
        dwq_v[:, :, cols] = _mm(xn_b, dq_b, TN).astype(BF16).reshape(dwq_v.shape[0], -1, GW)
        return s, dxn + _mm(dq_b, wq_v[:, :, cols].reshape(D, GW), NT)

    s, dxn = lax.fori_loop(0, HKV, kv_head, (zero, zero))
    write_batch(STREAMS[0], 0, False)
    out_v[...] = (x + s * g).astype(BF16)

    dbo = go * s * (sig * (1.0 + bo * (1.0 - sig)))
    dbo_b = dbo.astype(BF16)

    def ff_bwd(j, dln2):
        write_batch(STREAMS[0], j + 1, False)
        cols = _ds(j * FB, FB)
        u = u_s[j]
        t = _gelu_tanh(u)
        a = 0.5 * u * (1.0 + t)
        dgelu = 0.5 * (1.0 + t) + 0.5 * u * (1.0 - t * t) * GELU_C * (1.0 + 3.0 * GELU_A * u * u)
        du_b = (_mm(dbo_b, _row_block(w4_v, j, FB)[...], NT) * dgelu).astype(BF16)
        _row_block(dw4_v, j, FB)[...] = _mm(a.astype(BF16), dbo_b, TN).astype(BF16)
        dw3_v[:, :, cols] = _mm(ln2_b, du_b, TN).astype(BF16).reshape(dw3_v.shape[0], -1, FB)
        return dln2 + _mm(du_b, w3_v[:, :, cols].reshape(D, FB), NT)

    dln2 = lax.fori_loop(0, NF, ff_bwd, zero)
    write_batches(STREAMS[0], NF + 1, WINDOW_BATCHES, False)
    dxn = dxn + dbo + _layernorm_bwd(dln2, ln2, rstd2)
    dx_v[...] = (go + _layernorm_bwd(dxn, xn, rstd1)).astype(BF16)

    write_batches(STREAMS[1], 0, WINDOW_BATCHES, False)
    write_batches(STREAMS[2], 0, ZERO_BATCHES, True)
    write_batches(STREAMS[2], 0, WINDOW_BATCHES, False)
    pltpu.make_async_copy(out_v, out_hbm, write_sem).start()
    pltpu.make_async_copy(dx_v, dx_hbm, write_sem).start()
    _copy_matrices(((dwq_v, dwq_hbm, WRITE_PIECE), (dwo_v, dwo_hbm, WRITE_PIECE)),
                   write_sem, (0, 0))
    _copy_matrices(((dw3_v, dw3_hbm, WRITE_PIECE), (dw4_v, dw4_hbm, WRITE_PIECE)),
                   write_sem, (0, 0))

    for ref in (out_hbm, dx_hbm, dwq_hbm, dwo_hbm, dw3_hbm, dw4_hbm, dk_hbm, dv_hbm):
        _wait(ref, write_sem)


@jax.jit
def pallas_recurrent_scan__sliding_block_cached__mixer_s_mlp__decode_kernel(
    A_x: jax.Array,
    A_k_cache: jax.Array,
    A_v_cache: jax.Array,
    A_wq: jax.Array,
    A_wo: jax.Array,
    B_x: jax.Array,
    B_w1: jax.Array,
    B_w2: jax.Array,
    B_w3: jax.Array,
    B_w4: jax.Array,
    grad_out: jax.Array,
):
    assert A_x.shape == (NB, 1, D) and A_k_cache.shape == (NB, HKV, SK, DH)
    read_shapes = [(g, r // g, c) for g, (r, c) in zip(READ_GROUPS, MATRICES)]
    write_shapes = [(g, r // g, c) for g, (r, c) in zip(WRITE_GROUPS, MATRICES)]
    hbm = pl.BlockSpec(memory_space=pltpu.HBM)

    def vmem(shapes, dtype=BF16):
        return [pltpu.VMEM(shape, dtype) for shape in shapes]

    outs = pl.pallas_call(
        _kernel,
        in_specs=[hbm] * 8,
        out_specs=[hbm] * 8,
        out_shape=[
            jax.ShapeDtypeStruct(shape, BF16)
            for shape in [(NB, D)] * 2 + [(NS, NC, SK, DH)] * 2 + write_shapes
        ],
        scratch_shapes=[
            *vmem([(NB, D)] * 2 + [(NB, HKV, W, DH)] * 2 + read_shapes),
            *vmem([(NB, D)] * 2 + [(NS, NC, W, DH)] * 2 + write_shapes),
            *vmem([(max(n for streams in STREAMS for _, _, n in streams), ROWS, DH)]),
            *vmem([(NF, NB, FB)] + [(NB, 8, DH)] * 4, F32),
            pltpu.SemaphoreType.DMA((2,)),
        ],
        compiler_params=pltpu.CompilerParams(
            vmem_limit_bytes=110 * 2**20, disable_bounds_checks=True),
    )(
        A_x.reshape(NB, D), A_k_cache, A_v_cache,
        *[w.reshape(shape) for w, shape in zip((A_wq, A_wo, B_w3, B_w4), read_shapes)],
        grad_out.reshape(NB, D),
    )
    like = (A_x, A_x, A_k_cache, A_v_cache, A_wq, A_wo, B_w3, B_w4)
    return tuple(o.reshape(a.shape) for o, a in zip(outs, like))
```
